```python
import os as _os
_os.environ.setdefault('JAX_PLATFORMS', 'cpu')
import jax
import jax.numpy as jnp

def _softmax(x, axis=-1):
    return jax.nn.softmax(x, axis=axis)

def _gelu(x):
    return jax.nn.gelu(x, approximate=True)

def _silu(x):
    return jax.nn.silu(x)

def _sigmoid(x):
    return jax.nn.sigmoid(x)

def _layernorm(x, axis=-1, eps=1e-05):
    m = jnp.mean(x, axis=axis, keepdims=True)
    v = jnp.var(x, axis=axis, keepdims=True)
    return (x - m) / jnp.sqrt(v + eps)

def _scatter_add(tgt, idx, src, axis=0):
    return tgt.at[idx].add(src)

def _segment_sum(src, seg, n):
    return jax.ops.segment_sum(src, seg, n)

class _Rng:

    def __init__(self, key):
        self._k = key

    def _next(self):
        self._k, sub = jax.random.split(self._k)
        return sub

    def normal(self, shape):
        return jax.random.normal(self._next(), shape, dtype=jnp.bfloat16)

    def randint(self, lo, hi, shape):
        return jax.random.randint(self._next(), shape, lo, hi, dtype=jnp.int32)

    def uniform(self, shape, lo=0.0, hi=1.0):
        return jax.random.uniform(self._next(), shape, jnp.bfloat16, lo, hi)

    def permutation(self, n):
        return jax.random.permutation(self._next(), n)
kernel_name = 'adaLN_cond__sliding_local_dilated__dense_activation_relu__prompt'

def setup_inputs():
    _rng = _Rng(jax.random.key(int.from_bytes(__import__("os").urandom(4), "little")))
    _w = lambda a: (lambda t: t.astype(jnp.bfloat16) if jnp.issubdtype(t.dtype, jnp.floating) else t)(jnp.asarray(a))

    def _A_setup():
        B, S, D = (1, 2048, 576)
        return {'x': _w((lambda *s: _rng.normal(s) * 0.05)(B, S, D)), 'wqkv': _w((lambda *s: _rng.normal(s) * 0.05)(D, 3 * D)), 'wo': _w((lambda *s: _rng.normal(s) * 0.05)(D, D))}
    _A_in = _A_setup()

    def _B_setup():
        B, S, D, Dff = (1, 2048, 576, 4608)
        return {'x': _w((lambda *s: _rng.normal(s) * 0.05)(B, S, D)), 'w1': _w((lambda *s: _rng.normal(s) * 0.05)(D, Dff)), 'w2': _w((lambda *s: _rng.normal(s) * 0.05)(Dff, D))}
    _B_in = _B_setup()
    return {'A_x': _A_in['x'], 'A_wqkv': _A_in['wqkv'], 'A_wo': _A_in['wo'], 'B_x': _B_in['x'], 'B_w1': _B_in['w1'], 'B_w2': _B_in['w2'], 'c': _w((lambda *s: _rng.normal(s) * 0.05)(1, 576) * 8.0), 'w_mod': _w((lambda *s: _rng.normal(s) * 0.05)(576, 6 * 576) * 576 ** (-0.5) * 8.0)}

def reference(A_x, A_wqkv, A_wo, B_x, B_w1, B_w2, c, w_mod):

    def _A_ref(x, wqkv, wo):
        B, S, D = x.shape
        H = 32
        Dh = D // H
        W, dil = (8, 2)
        qkv = (lambda x, *d: x.transpose(*d))((x @ wqkv).reshape(B, S, 3, H, Dh), 2, 0, 3, 1, 4)
        q, k, v = (qkv[0], qkv[1], qkv[2])
        scale = Dh ** (-0.5)
        pos = jnp.arange(S)
        off = jnp.arange(W) * dil
        idx = pos[:, None] - off[None, :]
        mask = idx >= 0
        idx_c = jnp.where(mask, idx, 0).reshape(-1)
        kg = k[:, :, idx_c, :].reshape(B, H, S, W, Dh)
        vg = v[:, :, idx_c, :].reshape(B, H, S, W, Dh)
        logits = jnp.einsum('bhsd,bhswd->bhsw', q, kg) * scale
        logits = jnp.where(mask[None, None, :, :], logits, -1000000000.0)
        attn = _softmax(logits, axis=-1)
        o = jnp.einsum('bhsw,bhswd->bhsd', attn, vg)
        return (lambda x, *d: x.transpose(*d))(o, 0, 2, 1, 3).reshape(B, S, D) @ wo

    def _B_ref(x, w1, w2):
        h = jnp.einsum('bsd,df->bsf', x, w1)
        zero = jnp.zeros_like(h)
        h = jnp.maximum(h, zero)
        return jnp.einsum('bsf,fd->bsd', h, w2)
    x = A_x
    mod = (_silu(c) @ w_mod).reshape(c.shape[0], 6, 1, -1)
    sa, ca, ga, sb, cb, gb = (mod[:, 0].copy(), mod[:, 1].copy(), mod[:, 2].copy(), mod[:, 3].copy(), mod[:, 4].copy(), mod[:, 5].copy())
    h = _layernorm(x, axis=-1) * (1 + ca) + sa
    x = x + ga * _A_ref(h, A_wqkv, A_wo)
    h = _layernorm(x, axis=-1) * (1 + cb) + sb
    x = x + gb * _B_ref(h, B_w1, B_w2)
    return x
```

```python
import math
import jax
import jax.numpy as jnp
from jax import lax
import jax.experimental.pallas as pl
import jax.experimental.pallas.tpu as pltpu

S, D, H, DH, W, DIL, DFF = 2048, 576, 32, 18, 8, 2, 4608
TM = 256
TQ = 256
FC = 512
RG = 16
NB = S // TM
NQB = S // TQ
QPM = TM // TQ
NF = DFF // FC
HALO = 16
NQ = 14 * 128
KO = 5 * 128
f32 = jnp.float32
bf16 = jnp.bfloat16
NTD = (((1,), (1,)), ((), ()))
Q0 = 0
KV0 = Q0 + 5 * S
KVP = HALO + S
ACC0 = KV0 + 9 * KVP
BIG_ROWS = ACC0 + 2 * (TM // 128) * D


def _qkv_row(s, d):
    if d < 16:
        return (0, 5, 9)[s] * 128 + d * 32
    return ((4 * 128, 13 * 128, 13 * 128 + 64)[s]) + (d - 16) * 32


def _ln_rows(load, g_of, s_of):
    CH = 16
    def col_sum(fn):
        accs = [None, None]
        for i, r in enumerate(range(0, D, CH)):
            t = fn(load(r, CH))
            t = t[0:8, :] + t[8:16, :]
            accs[i % 2] = t if accs[i % 2] is None else accs[i % 2] + t
        return jnp.sum(accs[0] + accs[1], axis=0, keepdims=True) * (1.0 / D)
    m = col_sum(lambda x: x)
    v = col_sum(lambda x: (x - m) * (x - m))
    rstd = lax.rsqrt(v + 1e-5)
    outs = []
    for r in range(0, D, CH):
        outs.append((((load(r, CH) - m) * rstd) * g_of(r, CH) + s_of(r, CH)).astype(bf16))
    return jnp.concatenate(outs, axis=0)


def _mul(a, b):
    r = a * b
    if not isinstance(r, int):
        r = pl.multiple_of(r, b)
    return r


def kernel(c_hbm, wmod_hbm, xT_hbm, wqkv_hbm, wo_hbm, w1_hbm, w2T_hbm, outT_hbm,
           c_v, wmod_v, x_v, out_v, wqkv_v, wo_v, w1_v, w2T_v,
           modT_v, wt32_v, wqkvT_v, wo32_v, woT_v,
           h_v, h2_v, o_v, big_v, x1_v, z_ref, sem, osem):
    def cp(i, src, dst):
        return pltpu.make_async_copy(src, dst, sem.at[i])
    d_c = cp(0, c_hbm, c_v)
    d_modA = cp(1, wmod_hbm.at[:, pl.ds(0, 2 * D)], wmod_v.at[:, pl.ds(0, 2 * D)])
    d_modB = cp(2, wmod_hbm.at[:, pl.ds(2 * D, 4 * D)], wmod_v.at[:, pl.ds(2 * D, 4 * D)])
    d_wqkv = cp(3, wqkv_hbm, wqkv_v)
    d_wo = cp(4, wo_hbm, wo_v)
    d_w1 = cp(5, w1_hbm, w1_v)
    d_w2 = cp(6, w2T_hbm, w2T_v)
    d_x = [cp(7 + b, xT_hbm.at[:, pl.ds(b * TQ, TQ)], x_v.at[b]) for b in range(NQB)]

    DM = 'b'
    if DM == 'a':
        first = [d_c, d_modA, d_x[0], d_wqkv, d_x[1]]
    else:
        first = [d_wqkv, d_c, d_modA, d_x[0], d_x[1]]
    for d in first + d_x[2:] + [d_wo, d_modB, d_w1, d_w2]:
        d.start()

    def mod_part(col0, ncol):
        c = c_v[...].astype(f32)
        s = (c * jax.nn.sigmoid(c)).astype(bf16)
        s8 = jnp.broadcast_to(s, (8, D))
        m = jnp.dot(s8, wmod_v[:, col0:col0 + ncol], preferred_element_type=f32)
        col = col0 + lax.broadcasted_iota(jnp.int32, (1, ncol), 1)
        is_scale = ((col >= D) & (col < 2 * D)) | ((col >= 4 * D) & (col < 5 * D))
        m1 = jnp.where(is_scale, m[0:1, :] + 1.0, m[0:1, :])
        modT_v[col0:col0 + ncol, :] = jnp.broadcast_to(m1, (128, ncol)).T

    rep = lambda j: jnp.tile(modT_v[j * D:(j + 1) * D, :], (1, TM // 128))
    repc = lambda j, nt: (lambda r, n: jnp.tile(modT_v[j * D + r:j * D + r + n, :], (1, nt)))

    def stage_L(b, h_v):
        hT = _ln_rows(lambda r, n: x_v[b, r:r + n, :].astype(f32), repc(1, TQ // 128), repc(0, TQ // 128))
        h_v[...] = hT.T

    def stage_Q(b, h_v, t0=0, t1=14):
        r = _mul(b, TQ)
        qkv = lax.dot_general(h_v[...], wqkvT_v[t0 * 128:t1 * 128, 0:D], NTD, preferred_element_type=f32)
        for t in range(t0, t1):
            dst = Q0 + t * S if t < 5 else KV0 + (t - 5) * KVP + HALO
            big_v[pl.ds(dst + r, TQ), :] = qkv[:, (t - t0) * 128:(t - t0 + 1) * 128]

    cexp = (DH ** -0.5) * math.log2(math.e)

    def stage_B(b, g):
        static_g = isinstance(g, int)
        r0 = _mul(b, TM) + _mul(g, RG)
        kv = lambda t, off: big_v[pl.ds(KV0 + t * KVP + off + r0, RG), :]
        q = [big_v[pl.ds(Q0 + t * S + r0, RG), :] for t in range(5)]
        ls = []
        for w in range(W):
            off = HALO - DIL * w
            acc = None
            for t in range(5):
                p = q[t] * kv(t if t < 4 else 8, off)
                acc = p if acc is None else acc + p
            acc = acc + pltpu.roll(acc, 64, 1)
            acc = acc + pltpu.roll(acc, 32, 1)
            if w > 0 and (not static_g or g * RG < DIL * w):
                row = r0 + lax.broadcasted_iota(jnp.int32, (RG, 128), 0)
                acc = jnp.where(row >= DIL * w, acc, -1e9)
            ls.append(acc)
        mx = ls[0]
        for w in range(1, W):
            mx = jnp.maximum(mx, ls[w])
        es = [jnp.exp2((l - mx) * cexp) for l in ls]
        sm = es[0]
        for w in range(1, W):
            sm = sm + es[w]
        inv = 1.0 / sm
        for t in range(5):
            acc = None
            for w in range(W):
                off = HALO - DIL * w
                p = es[w] * kv(4 + t if t < 4 else 8, off)
                acc = p if acc is None else acc + p
            o_v[pl.ds(_mul(g, RG), RG), t * 128:(t + 1) * 128] = (acc * inv).astype(bf16)

    def stage_O(b, slot):
        a = lax.dot_general(woT_v[...], o_v[...], NTD, preferred_element_type=f32)
        x = jnp.concatenate([x_v[b * QPM + i] for i in range(QPM)], axis=1).astype(f32)
        x1_v[slot] = x + rep(2) * a

    def stage_N(slot):
        h2T = _ln_rows(lambda r, n: x1_v[slot, r:r + n, :], repc(4, TM // 128), repc(3, TM // 128))
        h2_v[slot] = h2T.T

    def acc_rows(slot, j):
        return pl.ds(ACC0 + _mul(slot, (TM // 128) * D) + j * D, D)

    def stage_F(slot, f):
        hh = jnp.dot(h2_v[slot], w1_v[:, f * FC:(f + 1) * FC], preferred_element_type=f32)
        hh = jnp.maximum(hh, 0.0).astype(bf16)
        p = lax.dot_general(w2T_v[:, f * FC:(f + 1) * FC], hh, NTD, preferred_element_type=f32)
        for j in range(TM // 128):
            if f == 0:
                big_v[acc_rows(slot, j), :] = p[:, j * 128:(j + 1) * 128]
            else:
                big_v[acc_rows(slot, j), :] += p[:, j * 128:(j + 1) * 128]

    def out_copy(b, slot):
        return pltpu.make_async_copy(out_v.at[slot], outT_hbm.at[:, pl.ds(_mul(b, TM), TM)], osem.at[slot])

    def stage_out(slot):
        acc = jnp.concatenate([big_v[acc_rows(slot, j), :] for j in range(TM // 128)], axis=1)
        out_v[slot] = (x1_v[slot] + rep(5) * acc).astype(bf16)

    def build_wqkv():
        wt = wqkv_v[...].T.astype(f32)
        for kt in range(5):
            n = min(128, D - kt * 128)
            blk = wt[:, kt * 128:kt * 128 + n]
            if n < 128:
                blk = jnp.concatenate([blk, jnp.zeros((3 * D, 128 - n), f32)], axis=1)
            wt32_v[kt] = blk
        wqkvT_v[4 * 128 + 64:5 * 128, :] = jnp.zeros((64, KO), bf16)
        for kt in range(5):
            for s in range(3):
                for d in range(DH):
                    rows = [wt32_v[kt, pl.ds(s * D + DH * 8 * hg + d, 8, stride=DH), :] for hg in range(4)]
                    c0 = _qkv_row(s, d)
                    wqkvT_v[c0:c0 + 32, kt * 128:(kt + 1) * 128] = jnp.concatenate(rows, axis=0).astype(bf16)

    def build_wo():
        w = wo_v[...].astype(f32)
        for nt in range(5):
            n = min(128, D - nt * 128)
            blk = w[:, nt * 128:nt * 128 + n]
            if n < 128:
                blk = jnp.concatenate([blk, jnp.zeros((D, 128 - n), f32)], axis=1)
            wo32_v[nt] = blk
        for nt in range(5):
            n = min(128, D - nt * 128)
            tiles = []
            for t in range(5):
                parts = []
                for dd in range(4):
                    if t < 4:
                        d = 4 * t + dd
                    elif dd >= 2:
                        d = 16 + dd - 2
                    else:
                        parts.append(jnp.zeros((32, 128), f32))
                        continue
                    parts += [wo32_v[nt, pl.ds(DH * 8 * hg + d, 8, stride=DH), :] for hg in range(4)]
                tiles.append(jnp.concatenate(parts, axis=0).astype(bf16))
            blk = jnp.concatenate(tiles, axis=0)
            woT_v[nt * 128:nt * 128 + n, :] = blk.T[0:n, :]

    nB = TM // RG
    z_ref[0] = 0
    for t in range(9):
        big_v[KV0 + t * KVP:KV0 + t * KVP + HALO, :] = jnp.zeros((HALO, 128), f32)
    for j in range(TM // 128):
        big_v[acc_rows(0, j), :] = jnp.zeros((D, 128), f32)
    x1_v[0] = jnp.zeros((D, TM), f32)
    if DM == 'a':
        d_c.wait(); d_modA.wait()
        mod_part(0, 2 * D)
        d_x[0].wait()
        stage_L(0, h_v.at[0])
        d_wqkv.wait(); d_x[1].wait()
        build_wqkv()
    else:
        d_wqkv.wait()
        build_wqkv()
        d_c.wait(); d_modA.wait(); d_x[0].wait(); d_x[1].wait()
        mod_part(0, 2 * D)
        stage_L(0, h_v.at[0])
    stage_L(1, h_v.at[1])
    stage_Q(0, h_v.at[0])
    for b in range(2, NQB):
        d_x[b].wait()
    d_wo.wait()
    z = z_ref[0]
    BM = 5
    B0 = 1
    B1 = NQB - 3
    gi = 0
    for b in range(1, NQB - 1):
        stage_L(b + 1, h_v.at[b + 1])
        stage_Q(b, h_v.at[b])
        if b == 1:
            build_wo()
        if b >= QPM * B0:
            gend = min(nB, (nB * (b + 1 - B0)) // (B1 + 1 - B0))
            while gi < gend:
                stage_B(z, gi)
                gi += 1
        if b == BM:
            d_modB.wait()
            mod_part(2 * D, 4 * D)
    assert gi == nB
    stage_O(0, 0)
    stage_Q(NQB - 1, h_v.at[NQB - 1])
    stage_N(0)
    d_w1.wait(); d_w2.wait()

    FO = 5
    FN = FO + 1
    def body(s, carry):
        cur = s % 2
        prv = 1 - cur
        sB = jnp.minimum(s, NB - 1)

        @pl.when(s >= 4)
        def _():
            out_copy(s - 4, cur).wait()

        @pl.when(s >= 3)
        def _():
            out_copy(s - 3, prv).start()

        gi = 0
        for f in range(NF):
            stage_F(prv, f)
            if f == 0:
                stage_out(cur)
            if f < FO:
                gend = min(nB, (nB * (f + 1)) // FO)
                while gi < gend:
                    stage_B(sB, gi)
                    gi += 1
            if f == FO:
                stage_O(sB, cur)
            if f == FN:
                stage_N(cur)
        return carry

    lax.fori_loop(1, NB + 1, body, 0)
    out_copy(NB - 3, (NB - 3) % 2).wait()
    out_copy(NB - 2, (NB - 2) % 2).start()
    stage_out((NB - 1) % 2)
    out_copy(NB - 1, (NB - 1) % 2).start()
    out_copy(NB - 2, (NB - 2) % 2).wait()
    out_copy(NB - 1, (NB - 1) % 2).wait()


@jax.jit
def pallas_adaLN_cond__sliding_local_dilated__dense_activation_relu__prompt_kernel(
    A_x, A_wqkv, A_wo, B_x, B_w1, B_w2, c, w_mod):
    xT = A_x.reshape(S, D).T
    w2T = B_w2.T
    anyspec = pl.BlockSpec(memory_space=pl.ANY)
    outT = pl.pallas_call(
        kernel,
        grid=(1,),
        in_specs=[anyspec] * 7,
        out_specs=anyspec,
        out_shape=jax.ShapeDtypeStruct((D, S), bf16),
        scratch_shapes=[
            pltpu.VMEM((1, D), bf16),
            pltpu.VMEM((D, 6 * D), bf16),
            pltpu.VMEM((NQB, D, TQ), bf16),
            pltpu.VMEM((2, D, TM), bf16),
            pltpu.VMEM((D, 3 * D), bf16),
            pltpu.VMEM((D, D), bf16),
            pltpu.VMEM((D, DFF), bf16),
            pltpu.VMEM((D, DFF), bf16),
            pltpu.VMEM((6 * D, 128), f32),
            pltpu.VMEM((5, 3 * D, 128), f32),
            pltpu.VMEM((NQ, KO), bf16),
            pltpu.VMEM((5, D, 128), f32),
            pltpu.VMEM((D, KO), bf16),
            pltpu.VMEM((NQB, TQ, D), bf16),
            pltpu.VMEM((2, TM, D), bf16),
            pltpu.VMEM((TM, KO), bf16),
            pltpu.VMEM((BIG_ROWS, 128), f32),
            pltpu.VMEM((2, D, TM), f32),
            pltpu.SMEM((1,), jnp.int32),
            pltpu.SemaphoreType.DMA((7 + NQB,)),
            pltpu.SemaphoreType.DMA((2,)),
        ],
        compiler_params=pltpu.CompilerParams(
            dimension_semantics=("arbitrary",),
            vmem_limit_bytes=100 * 1024 * 1024,
        ),
    )(c, w_mod, xT, A_wqkv, A_wo, B_w1, w2T)
    return outT.T.reshape(1, S, D)
```

```python
import math
import jax
import jax.numpy as jnp
from jax import lax
import jax.experimental.pallas as pl
import jax.experimental.pallas.tpu as pltpu

S, D, H, DH, W, DIL, DFF = 2048, 576, 32, 18, 8, 2, 4608
TM = 256
TQ = 256
FC = 512
RG = 32
NB = S // TM
NQB = S // TQ
QPM = TM // TQ
NF = DFF // FC
HALO = 16
NQ = 14 * 128
KO = 5 * 128
f32 = jnp.float32
bf16 = jnp.bfloat16
NTD = (((1,), (1,)), ((), ()))
Q0 = 0
QP = S + 16
KV0 = Q0 + 5 * QP
KVP = HALO + S + 8 + 0
NC = W // 2
PIN0 = KV0 + NC * 9 * KVP
BIG_ROWS = PIN0 + 8


def _qkv_row(s, d):
    if d < 16:
        return (0, 5, 9)[s] * 128 + d * 32
    return ((4 * 128, 13 * 128, 13 * 128 + 64)[s]) + (d - 16) * 32


def _ln_rows(load, g_of, s_of):
    CH = 16
    def col_sum(fn):
        accs = [None, None]
        for i, r in enumerate(range(0, D, CH)):
            t = fn(load(r, CH))
            t = t[0:8, :] + t[8:16, :]
            accs[i % 2] = t if accs[i % 2] is None else accs[i % 2] + t
        return jnp.sum(accs[0] + accs[1], axis=0, keepdims=True) * (1.0 / D)
    m = col_sum(lambda x: x)
    v = col_sum(lambda x: (x - m) * (x - m))
    rstd = lax.rsqrt(v + 1e-5)
    outs = []
    for r in range(0, D, CH):
        outs.append((((load(r, CH) - m) * rstd) * g_of(r, CH) + s_of(r, CH)).astype(bf16))
    return jnp.concatenate(outs, axis=0)


def _mul(a, b):
    r = a * b
    if not isinstance(r, int):
        r = pl.multiple_of(r, b)
    return r


def kernel(c_hbm, wmod_hbm, xT_hbm, wqkv_hbm, wo_hbm, w1_hbm, w2T_hbm, outT_hbm,
           c_v, wmod_v, x_v, out_v, wqkv_v, wo_v, w1_v, w2T_v,
           modT_v, wt32_v, wqkvT_v, wo32_v, woT_v,
           h_v, h2_v, o_v, hh_v, big_v, acc_v, x1_v, modS_v, z_ref, sem, osem):
    def cp(i, src, dst):
        return pltpu.make_async_copy(src, dst, sem.at[i])
    d_c = cp(0, c_hbm, c_v)
    d_modA = cp(1, wmod_hbm.at[:, pl.ds(0, 2 * D)], wmod_v.at[:, pl.ds(0, 2 * D)])
    d_modB = cp(2, wmod_hbm.at[:, pl.ds(2 * D, 4 * D)], wmod_v.at[:, pl.ds(2 * D, 4 * D)])
    WCH = ((0, 640), (640, 1152), (1152, 3 * D))
    d_wqkv = [cp(7 + NQB + i, wqkv_hbm.at[:, pl.ds(a, b - a)], wqkv_v.at[:, pl.ds(a, b - a)]) for i, (a, b) in enumerate(WCH)]
    d_wo = cp(4, wo_hbm, wo_v)
    d_w1 = cp(5, w1_hbm, w1_v)
    d_w2 = cp(6, w2T_hbm, w2T_v)
    d_x = [cp(7 + b, xT_hbm.at[:, pl.ds(b * TQ, TQ)], x_v.at[b]) for b in range(NQB)]

    for d in ([d_wqkv[0], d_c, d_modA, d_x[0], d_x[1], d_wqkv[1], d_wqkv[2]] + d_x[2:]
              + [d_wo, d_modB, d_w1, d_w2]):
        d.start()

    def mod_rows(col0, ncol):
        c = c_v[...].astype(f32)
        s = (c * jax.nn.sigmoid(c)).astype(bf16)
        return jnp.dot(jnp.broadcast_to(s, (8, D)), wmod_v[:, col0:col0 + ncol], preferred_element_type=f32)

    def mod_first():
        m = mod_rows(0, 2 * D)
        modS_v[0] = m[:, 0:D]
        modS_v[1] = m[:, D:2 * D] + 1.0

    def mod_part(col0, ncol):
        m = mod_rows(col0, ncol)
        col = col0 + lax.broadcasted_iota(jnp.int32, (1, ncol), 1)
        m1 = jnp.where((col >= 4 * D) & (col < 5 * D), m[0:1, :] + 1.0, m[0:1, :])
        modT_v[col0:col0 + ncol, :] = jnp.broadcast_to(m1, (128, ncol)).T

    rep = lambda j: jnp.tile(modT_v[j * D:(j + 1) * D, :], (1, TM // 128))
    repc = lambda j, nt: (lambda r, n: jnp.tile(modT_v[j * D + r:j * D + r + n, :], (1, nt)))

    def ld_tiles(ref, width):
        n = -(-width // 128)
        return jnp.concatenate([ref[t] for t in range(n)], axis=1)[:, 0:width]

    def st_tiles(ref, val):
        for t in range(-(-val.shape[1] // 128)):
            n = min(128, val.shape[1] - t * 128)
            ref[t, :, 0:n] = val[:, t * 128:t * 128 + n]

    LCH = 16
    def stage_L(b, h_v, z=0):
        x = x_v[b + z].T
        g = jnp.tile(modS_v[1], (LCH // 8, 1))
        sh = jnp.tile(modS_v[0], (LCH // 8, 1))
        for r in range(0, TQ, LCH):
            xf = x[r:r + LCH, :].astype(f32)
            xc = xf - jnp.mean(xf, axis=1, keepdims=True)
            v = jnp.mean(xc * xc, axis=1, keepdims=True)
            st_tiles(h_v.at[:, r:r + LCH, :], ((xc * lax.rsqrt(v + 1e-5)) * g + sh).astype(bf16))

    cexp = (DH ** -0.5) * math.log2(math.e)
    PINL = 0
    def stage_Q(b, h_v, t0=0, t1=14):
        r = _mul(b, TQ)
        qkv = lax.dot_general(ld_tiles(h_v, D), wqkvT_v[t0 * 128:t1 * 128, 0:D], NTD, preferred_element_type=f32)
        for t in range(t0, t1):
            val = qkv[:, (t - t0) * 128:(t - t0 + 1) * 128]
            if t == PINL:
                x_v[NQB, 0:16, 0:128] = val[0:16, :].astype(bf16)
            if t < 5:
                big_v[pl.ds(Q0 + t * QP + r, TQ), :] = val * cexp
            else:
                for c in range(NC):
                    big_v[pl.ds(KV0 + (c * 9 + t - 5) * KVP + HALO + DIL * c + r, TQ), :] = val

    def stage_B(b, g):
        static_g = isinstance(g, int)
        r0 = _mul(b, TM) + _mul(g, RG)
        half = W // 2

        def windows(t):
            out = [None] * W
            for c in range(half):
                v = big_v[pl.ds(KV0 + (c * 9 + t) * KVP + HALO - DIL * half + r0, RG + DIL * half), :]
                out[c + half] = v[0:RG]
                out[c] = v[DIL * half:DIL * half + RG]
            return out

        ls = [None] * W
        for t in range(5):
            q = big_v[pl.ds(Q0 + t * QP + r0, RG), :]
            kw = windows(t if t < 4 else 8)
            for w in range(W):
                p = q * kw[w]
                ls[w] = p if ls[w] is None else ls[w] + p
        for w in range(W):
            acc = ls[w] + pltpu.roll(ls[w], 64, 1)
            acc = acc + pltpu.roll(acc, 32, 1)
            if w > 0 and (not static_g or g * RG < DIL * w):
                row = r0 + lax.broadcasted_iota(jnp.int32, (RG, 128), 0)
                acc = jnp.where(row >= DIL * w, acc, -1e9)
            ls[w] = acc
        mx = ls[0]
        for w in range(1, W):
            mx = jnp.maximum(mx, ls[w])
        es = [jnp.exp2(l - mx) for l in ls]
        sm = es[0]
        for w in range(1, W):
            sm = sm + es[w]
        inv = 1.0 / sm
        for t in range(5):
            vw = windows(4 + t if t < 4 else 8)
            acc = es[0] * vw[0]
            for w in range(1, W):
                acc = acc + es[w] * vw[w]
            o_v[t, pl.ds(_mul(g, RG), RG), :] = (acc * inv).astype(bf16)

    def stage_O(b, slot):
        a = lax.dot_general(woT_v[...], ld_tiles(o_v, KO), NTD, preferred_element_type=f32)
        x = jnp.concatenate([x_v[b * QPM + i] for i in range(QPM)], axis=1).astype(f32)
        x1_v[slot] = x + rep(2) * a

    def stage_N(slot):
        h2T = _ln_rows(lambda r, n: x1_v[slot, r:r + n, :], repc(4, TM // 128), repc(3, TM // 128))
        st_tiles(h2_v.at[slot], h2T.T)

    def stage_F1(slot, f):
        hh = jnp.dot(ld_tiles(h2_v.at[slot], D), w1_v[:, f * FC:(f + 1) * FC], preferred_element_type=f32)
        hh = jnp.maximum(hh, 0.0).astype(bf16)
        for t in range(FC // 128):
            hh_v[f % 2, t] = hh[:, t * 128:(t + 1) * 128]

    NPIN = 1
    PINJ = 0
    def stage_F2(slot, f, after=None):
        hh = ld_tiles(hh_v.at[f % 2], FC)
        p = lax.dot_general(w2T_v[:, f * FC:(f + 1) * FC], hh, NTD, preferred_element_type=f32)
        rows = D // NPIN
        for j in range(TM // 128):
            val = p[:, j * 128:(j + 1) * 128]
            if f == 0:
                acc_v[slot, j] = val
            else:
                acc_v[slot, j] += val
            if after is not None and (PINJ < 0 or j == PINJ):
                for k in range(NPIN):
                    big_v[PIN0:PIN0 + 8, :] = val[(k + 1) * rows - 8:(k + 1) * rows, :]
                    after()

    def out_copy(b, slot):
        return pltpu.make_async_copy(out_v.at[slot], outT_hbm.at[:, pl.ds(_mul(b, TM), TM)], osem.at[slot])

    def stage_out(slot):
        acc = jnp.concatenate([acc_v[slot, j] for j in range(TM // 128)], axis=1)
        out_v[slot] = (x1_v[slot] + rep(5) * acc).astype(bf16)

    def build_wqkv(s):
        c0, c1 = WCH[s]
        wt = wqkv_v[:, c0:c1].T.astype(f32)
        for kt in range(5):
            n = min(128, D - kt * 128)
            blk = wt[:, kt * 128:kt * 128 + n]
            if n < 128:
                blk = jnp.concatenate([blk, jnp.zeros((c1 - c0, 128 - n), f32)], axis=1)
            wt32_v[kt, c0:c1, :] = blk
        if s == 0:
            wqkvT_v[4 * 128 + 64:5 * 128, :] = jnp.zeros((64, KO), bf16)
        for kt in range(5):
            for d in range(DH):
                rows = [wt32_v[kt, pl.ds(s * D + DH * 8 * hg + d, 8, stride=DH), :] for hg in range(4)]
                r0 = _qkv_row(s, d)
                wqkvT_v[r0:r0 + 32, kt * 128:(kt + 1) * 128] = jnp.concatenate(rows, axis=0).astype(bf16)

    def build_wo():
        w = wo_v[...].astype(f32)
        for nt in range(5):
            n = min(128, D - nt * 128)
            blk = w[:, nt * 128:nt * 128 + n]
            if n < 128:
                blk = jnp.concatenate([blk, jnp.zeros((D, 128 - n), f32)], axis=1)
            wo32_v[nt] = blk
        for nt in range(5):
            n = min(128, D - nt * 128)
            tiles = []
            for t in range(5):
                parts = []
                for dd in range(4):
                    if t < 4:
                        d = 4 * t + dd
                    elif dd >= 2:
                        d = 16 + dd - 2
                    else:
                        parts.append(jnp.zeros((32, 128), f32))
                        continue
                    parts += [wo32_v[nt, pl.ds(DH * 8 * hg + d, 8, stride=DH), :] for hg in range(4)]
                tiles.append(jnp.concatenate(parts, axis=0).astype(bf16))
            blk = jnp.concatenate(tiles, axis=0)
            woT_v[nt * 128:nt * 128 + n, :] = blk.T[0:n, :]

    nB = TM // RG
    z_ref[0] = 0
    for t in range(NC * 9):
        big_v[KV0 + t * KVP:KV0 + t * KVP + HALO + 8, :] = jnp.zeros((HALO + 8, 128), f32)
    for j in range(TM // 128):
        acc_v[0, j] = jnp.zeros((D, 128), f32)
    x1_v[0] = jnp.zeros((D, TM), f32)
    SO = 'c'
    d_wqkv[0].wait()
    build_wqkv(0)
    d_c.wait(); d_modA.wait()
    mod_first()
    d_x[0].wait()
    stage_L(0, h_v.at[0])
    d_x[1].wait()
    stage_Q(0, h_v.at[0], 0, 5)
    stage_L(1, h_v.at[1])
    if SO == 'd':
        stage_Q(1, h_v.at[1], 0, 5)
    d_wqkv[1].wait(); d_wqkv[2].wait()
    if SO == 'c':
        stage_Q(1, h_v.at[1], 0, 5)
    build_wqkv(1)
    stage_Q(0, h_v.at[0], 5, 9)
    build_wqkv(2)
    stage_Q(0, h_v.at[0], 9, 14)
    for b in range(3 if SO == 'b' else 2, NQB):
        d_x[b].wait()
    d_wo.wait()
    z = z_ref[0]
    B0 = 1
    B1 = NQB - 3
    LZ = 1
    gi = 0
    for b in range(1, NQB - 1):
        if not LZ or b == 1:
            stage_L(b + 1, h_v.at[b + 1])
        stage_Q(b, h_v.at[b], 5 if b == 1 else 0)
        if LZ and b + 2 < NQB:
            stage_L(b + 2, h_v.at[b + 2], z)
        if b == 1:
            build_wo()
        if b >= QPM * B0:
            gend = min(nB, (nB * (b + 1 - B0)) // (B1 + 1 - B0))
            while gi < gend:
                stage_B(z, gi)
                gi += 1
    assert gi == nB
    d_modB.wait(); d_w1.wait(); d_w2.wait()
    mod_part(2 * D, 4 * D)
    stage_O(0, 0)
    stage_Q(NQB - 1, h_v.at[NQB - 1])
    stage_N(0)

    FO = 5
    FN = FO + 2
    def body(s, carry):
        cur = s % 2
        prv = 1 - cur
        sB = jnp.minimum(s, NB - 1)

        @pl.when(s >= 4)
        def _():
            out_copy(s - 4, cur).wait()

        gi = [0]
        npin = [0]
        PB0 = 0
        PB1 = FO * NPIN * (TM // 128 if PINJ < 0 else 1)
        def attn():
            npin[0] += 1
            if npin[0] <= PB0:
                return
            gend = min(nB, (nB * (npin[0] - PB0)) // (PB1 - PB0))
            while gi[0] < gend:
                stage_B(sB, gi[0])
                gi[0] += 1
        stage_F1(prv, 0)
        for f in range(NF):
            if f + 1 < NF:
                stage_F1(prv, f + 1)
            stage_F2(prv, f, attn)
            if f == 0:
                stage_out(cur)
            if f == 1:
                @pl.when(s >= 2)
                def _():
                    out_copy(s - 2, cur).start()
            if f == FO:
                assert gi[0] == nB
                stage_O(sB, cur)
            if f == FN:
                stage_N(cur)
        return carry

    lax.fori_loop(1, NB + 1, body, 0)
    out_copy(NB - 3, (NB - 3) % 2).wait()
    stage_out((NB - 1) % 2)
    out_copy(NB - 1, (NB - 1) % 2).start()
    out_copy(NB - 2, (NB - 2) % 2).wait()
    out_copy(NB - 1, (NB - 1) % 2).wait()


@jax.jit
def pallas_adaLN_cond__sliding_local_dilated__dense_activation_relu__prompt_kernel(
    A_x, A_wqkv, A_wo, B_x, B_w1, B_w2, c, w_mod):
    xT = A_x.reshape(S, D).T
    w2T = B_w2.T
    anyspec = pl.BlockSpec(memory_space=pl.ANY)
    outT = pl.pallas_call(
        kernel,
        grid=(1,),
        in_specs=[anyspec] * 7,
        out_specs=anyspec,
        out_shape=jax.ShapeDtypeStruct((D, S), bf16),
        scratch_shapes=[
            pltpu.VMEM((1, D), bf16),
            pltpu.VMEM((D, 6 * D), bf16),
            pltpu.VMEM((NQB + 1, D, TQ), bf16),
            pltpu.VMEM((2, D, TM), bf16),
            pltpu.VMEM((D, 3 * D), bf16),
            pltpu.VMEM((D, D), bf16),
            pltpu.VMEM((D, DFF), bf16),
            pltpu.VMEM((D, DFF), bf16),
            pltpu.VMEM((6 * D, 128), f32),
            pltpu.VMEM((5, 3 * D, 128), f32),
            pltpu.VMEM((NQ, KO), bf16),
            pltpu.VMEM((5, D, 128), f32),
            pltpu.VMEM((D, KO), bf16),
            pltpu.VMEM((NQB, 5, TQ, 128), bf16),
            pltpu.VMEM((2, 5, TM, 128), bf16),
            pltpu.VMEM((5, TM, 128), bf16),
            pltpu.VMEM((2, FC // 128, TM, 128), bf16),
            pltpu.VMEM((BIG_ROWS, 128), f32),
            pltpu.VMEM((2, TM // 128, D, 128), f32),
            pltpu.VMEM((2, D, TM), f32),
            pltpu.VMEM((2, 8, D), f32),
            pltpu.SMEM((1,), jnp.int32),
            pltpu.SemaphoreType.DMA((10 + NQB,)),
            pltpu.SemaphoreType.DMA((2,)),
        ],
        compiler_params=pltpu.CompilerParams(
            dimension_semantics=("arbitrary",),
            vmem_limit_bytes=110 * 1024 * 1024,
        ),
    )(c, w_mod, xT, A_wqkv, A_wo, B_w1, w2T)
    return outT.T.reshape(1, S, D)
```

```python
import math

import jax
import jax.numpy as jnp
from jax import lax
import jax.experimental.pallas as pl
import jax.experimental.pallas.tpu as pltpu

S, D, H, DH, W, DIL, DFF = 2048, 576, 32, 18, 8, 2, 4608
TM = 256
FC = 512
RG = 16
NB = S // TM
NT = TM // 128
NF = DFF // FC
HALO = 16
NQ = 14 * 128
KO = 5 * 128
NC = W // 2
f32 = jnp.float32
bf16 = jnp.bfloat16
NTD = (((1,), (1,)), ((), ()))
QP = S + 16
KV0 = 5 * QP
KVP = HALO + S + 8
PIN0 = KV0 + NC * 9 * KVP
QKV_ROWS = PIN0 + 8
WCH = ((0, 640), (640, 1152), (1152, 3 * D))
FO, FN = 5, 7


def _qkv_row(s, d):
    if d < 16:
        return (0, 5, 9)[s] * 128 + d * 32
    return (4 * 128, 13 * 128, 13 * 128 + 64)[s] + (d - 16) * 32


def _mul(a, b):
    r = a * b
    if not isinstance(r, int):
        r = pl.multiple_of(r, b)
    return r


def _ld_tiles(ref, width):
    n = -(-width // 128)
    return jnp.concatenate([ref[t] for t in range(n)], axis=1)[:, 0:width]


def _st_tiles(ref, val):
    for t in range(-(-val.shape[1] // 128)):
        n = min(128, val.shape[1] - t * 128)
        ref[t, :, 0:n] = val[:, t * 128:t * 128 + n]


def _kernel(c_hbm, wmod_hbm, xT_hbm, wqkv_hbm, wo_hbm, w1_hbm, w2T_hbm, outT_hbm,
            c_v, wmod_v, x_v, out_v, wqkv_v, wo_v, w1_v, w2T_v,
            modT_v, wt32_v, wqkvT_v, wo32_v, woT_v,
            h_v, h2_v, o_v, hh_v, qkv_v, acc_v, x1_v, modS_v, z_ref, sem, osem):
    def cp(i, src, dst):
        return pltpu.make_async_copy(src, dst, sem.at[i])
    d_c = cp(0, c_hbm, c_v)
    d_modA = cp(1, wmod_hbm.at[:, pl.ds(0, 2 * D)], wmod_v.at[:, pl.ds(0, 2 * D)])
    d_modB = cp(2, wmod_hbm.at[:, pl.ds(2 * D, 4 * D)], wmod_v.at[:, pl.ds(2 * D, 4 * D)])
    d_wo = cp(3, wo_hbm, wo_v)
    d_w1 = cp(4, w1_hbm, w1_v)
    d_w2 = cp(5, w2T_hbm, w2T_v)
    d_wqkv = [cp(6 + i, wqkv_hbm.at[:, pl.ds(a, b - a)], wqkv_v.at[:, pl.ds(a, b - a)])
              for i, (a, b) in enumerate(WCH)]
    d_x = [cp(9 + b, xT_hbm.at[:, pl.ds(b * TM, TM)], x_v.at[b]) for b in range(NB)]
    for d in ([d_wqkv[0], d_c, d_modA, d_x[0], d_x[1], d_wqkv[1], d_wqkv[2]] + d_x[2:]
              + [d_wo, d_modB, d_w1, d_w2]):
        d.start()

    def out_copy(b, slot):
        return pltpu.make_async_copy(out_v.at[slot], outT_hbm.at[:, pl.ds(_mul(b, TM), TM)], osem.at[slot])

    def mod_rows(col0, ncol):
        c = c_v[...].astype(f32)
        s = (c * jax.nn.sigmoid(c)).astype(bf16)
        return jnp.dot(jnp.broadcast_to(s, (8, D)), wmod_v[:, col0:col0 + ncol], preferred_element_type=f32)

    def mod_first():
        m = mod_rows(0, 2 * D)
        modS_v[0] = m[:, 0:D]
        modS_v[1] = m[:, D:2 * D] + 1.0

    def mod_rest():
        col0, ncol = 2 * D, 4 * D
        m = mod_rows(col0, ncol)
        col = col0 + lax.broadcasted_iota(jnp.int32, (1, ncol), 1)
        m1 = jnp.where((col >= 4 * D) & (col < 5 * D), m[0:1, :] + 1.0, m[0:1, :])
        modT_v[...] = jnp.broadcast_to(m1, (128, ncol)).T

    def col(j, r=0, n=D):
        return jnp.tile(modT_v[(j - 2) * D + r:(j - 2) * D + r + n, :], (1, NT))

    def build_wqkv(s):
        c0, c1 = WCH[s]
        wt = wqkv_v[:, c0:c1].T.astype(f32)
        for kt in range(5):
            n = min(128, D - kt * 128)
            blk = wt[:, kt * 128:kt * 128 + n]
            if n < 128:
                blk = jnp.concatenate([blk, jnp.zeros((c1 - c0, 128 - n), f32)], axis=1)
            wt32_v[kt, c0:c1, :] = blk
        if s == 0:
            wqkvT_v[4 * 128 + 64:5 * 128, :] = jnp.zeros((64, KO), bf16)
        for kt in range(5):
            for d in range(DH):
                rows = [wt32_v[kt, pl.ds(s * D + DH * 8 * hg + d, 8, stride=DH), :] for hg in range(4)]
                r0 = _qkv_row(s, d)
                wqkvT_v[r0:r0 + 32, kt * 128:(kt + 1) * 128] = jnp.concatenate(rows, axis=0).astype(bf16)

    def build_wo():
        w = wo_v[...].astype(f32)
        for nt in range(5):
            n = min(128, D - nt * 128)
            blk = w[:, nt * 128:nt * 128 + n]
            if n < 128:
                blk = jnp.concatenate([blk, jnp.zeros((D, 128 - n), f32)], axis=1)
            wo32_v[nt] = blk
        for nt in range(5):
            n = min(128, D - nt * 128)
            parts = []
            for t in range(5):
                for dd in range(4):
                    if t == 4 and dd < 2:
                        parts.append(jnp.zeros((32, 128), f32))
                        continue
                    d = 4 * t + dd if t < 4 else 14 + dd
                    parts += [wo32_v[nt, pl.ds(DH * 8 * hg + d, 8, stride=DH), :] for hg in range(4)]
            blk = jnp.concatenate(parts, axis=0).astype(bf16)
            woT_v[nt * 128:nt * 128 + n, :] = blk.T[0:n, :]

    def stage_ln1(b, z=0):
        x = x_v[b + z].T
        g = jnp.tile(modS_v[1], (2, 1))
        sh = jnp.tile(modS_v[0], (2, 1))
        for r in range(0, TM, 16):
            xf = x[r:r + 16, :].astype(f32)
            xc = xf - jnp.mean(xf, axis=1, keepdims=True)
            v = jnp.mean(xc * xc, axis=1, keepdims=True)
            _st_tiles(h_v.at[b, :, r:r + 16, :], ((xc * lax.rsqrt(v + 1e-5)) * g + sh).astype(bf16))

    cexp = (DH ** -0.5) * math.log2(math.e)

    def stage_qkv(b, t0=0, t1=14):
        r = b * TM
        qkv = lax.dot_general(_ld_tiles(h_v.at[b], D), wqkvT_v[t0 * 128:t1 * 128, 0:D], NTD,
                              preferred_element_type=f32)
        for t in range(t0, t1):
            val = qkv[:, (t - t0) * 128:(t - t0 + 1) * 128]
            if t == 0:
                x_v[NB, 0:16, 0:128] = val[0:16, :].astype(bf16)
            if t < 5:
                qkv_v[pl.ds(t * QP + r, TM), :] = val * cexp
            else:
                for cc in range(NC):
                    qkv_v[pl.ds(KV0 + (cc * 9 + t - 5) * KVP + HALO + DIL * cc + r, TM), :] = val

    def stage_attn(b, g):
        r0 = _mul(b, TM) + g * RG

        def windows(t):
            out = [None] * W
            for cc in range(NC):
                v = qkv_v[pl.ds(KV0 + (cc * 9 + t) * KVP + HALO - DIL * NC + r0, RG + DIL * NC), :]
                out[cc + NC] = v[0:RG]
                out[cc] = v[DIL * NC:DIL * NC + RG]
            return out

        ls = [None] * W
        for t in range(5):
            q = qkv_v[pl.ds(t * QP + r0, RG), :]
            kw = windows(t if t < 4 else 8)
            for w in range(W):
                p = q * kw[w]
                ls[w] = p if ls[w] is None else ls[w] + p
        for w in range(W):
            acc = ls[w] + pltpu.roll(ls[w], 64, 1)
            acc = acc + pltpu.roll(acc, 32, 1)
            if g * RG < DIL * w:
                row = r0 + lax.broadcasted_iota(jnp.int32, (RG, 128), 0)
                acc = jnp.where(row >= DIL * w, acc, -1e9)
            ls[w] = acc
        mx = ls[0]
        for w in range(1, W):
            mx = jnp.maximum(mx, ls[w])
        es = [jnp.exp2(l - mx) for l in ls]
        sm = es[0]
        for w in range(1, W):
            sm = sm + es[w]
        inv = 1.0 / sm
        for t in range(5):
            vw = windows(4 + t if t < 4 else 8)
            acc = es[0] * vw[0]
            for w in range(1, W):
                acc = acc + es[w] * vw[w]
            o_v[t, g * RG:(g + 1) * RG, :] = (acc * inv).astype(bf16)

    def stage_proj(b, slot):
        a = lax.dot_general(woT_v[...], _ld_tiles(o_v, KO), NTD, preferred_element_type=f32)
        x1_v[slot] = x_v[b].astype(f32) + col(2) * a

    def stage_ln2(slot):
        def col_mean(fn):
            accs = [None, None]
            for i, r in enumerate(range(0, D, 16)):
                t = fn(x1_v[slot, r:r + 16, :])
                t = t[0:8, :] + t[8:16, :]
                accs[i % 2] = t if accs[i % 2] is None else accs[i % 2] + t
            return jnp.sum(accs[0] + accs[1], axis=0, keepdims=True) * (1.0 / D)
        m = col_mean(lambda x: x)
        rstd = lax.rsqrt(col_mean(lambda x: (x - m) * (x - m)) + 1e-5)
        outs = [(((x1_v[slot, r:r + 16, :] - m) * rstd) * col(4, r, 16) + col(3, r, 16)).astype(bf16)
                for r in range(0, D, 16)]
        _st_tiles(h2_v.at[slot], jnp.concatenate(outs, axis=0).T)

    def stage_up(slot, f):
        hh = jnp.dot(_ld_tiles(h2_v.at[slot], D), w1_v[:, f * FC:(f + 1) * FC], preferred_element_type=f32)
        hh = jnp.maximum(hh, 0.0).astype(bf16)
        for t in range(FC // 128):
            hh_v[f % 2, t] = hh[:, t * 128:(t + 1) * 128]

    def stage_down(slot, f, behind):
        p = lax.dot_general(w2T_v[:, f * FC:(f + 1) * FC], _ld_tiles(hh_v.at[f % 2], FC), NTD,
                            preferred_element_type=f32)
        for j in range(NT):
            val = p[:, j * 128:(j + 1) * 128]
            if f == 0:
                acc_v[slot, j] = val
            else:
                acc_v[slot, j] += val
            if j == 0:
                qkv_v[PIN0:PIN0 + 8, :] = val[D - 8:D, :]
                behind()

    def stage_out(slot):
        acc = jnp.concatenate([acc_v[slot, j] for j in range(NT)], axis=1)
        out_v[slot] = (x1_v[slot] + col(5) * acc).astype(bf16)

    nG = TM // RG
    z_ref[0] = 0
    for t in range(NC * 9):
        qkv_v[KV0 + t * KVP:KV0 + t * KVP + HALO + 8, :] = jnp.zeros((HALO + 8, 128), f32)
    for j in range(NT):
        acc_v[1, j] = jnp.zeros((D, 128), f32)
    x1_v[1] = jnp.zeros((D, TM), f32)
    d_wqkv[0].wait()
    build_wqkv(0)
    d_c.wait()
    d_modA.wait()
    mod_first()
    d_x[0].wait()
    stage_ln1(0)
    d_x[1].wait()
    stage_qkv(0, 0, 5)
    stage_ln1(1)
    d_wqkv[1].wait()
    d_wqkv[2].wait()
    stage_qkv(1, 0, 5)
    build_wqkv(1)
    stage_qkv(0, 5, 9)
    build_wqkv(2)
    stage_qkv(0, 9, 14)
    for b in range(2, NB):
        d_x[b].wait()
    d_wo.wait()
    z = z_ref[0]
    gi = 0
    stage_ln1(2)
    for b in range(1, NB - 1):
        stage_qkv(b, 5 if b == 1 else 0)
        if b + 2 < NB:
            stage_ln1(b + 2, z)
        if b == 1:
            build_wo()
        gend = min(nG, (nG * b) // (NB - 3))
        while gi < gend:
            stage_attn(z, gi)
            gi += 1
    d_modB.wait()
    d_w1.wait()
    d_w2.wait()
    mod_rest()
    stage_proj(0, 0)
    stage_qkv(NB - 1)
    stage_ln2(0)

    def body(s, carry):
        cur = s % 2
        prv = 1 - cur
        sB = jnp.minimum(s, NB - 1)

        @pl.when(s >= 4)
        def _():
            out_copy(s - 4, cur).wait()

        state = [0, 0]

        def attn():
            state[1] += 1
            gend = min(nG, (nG * state[1]) // FO)
            while state[0] < gend:
                stage_attn(sB, state[0])
                state[0] += 1

        stage_up(prv, 0)
        for f in range(NF):
            if f + 1 < NF:
                stage_up(prv, f + 1)
            stage_down(prv, f, attn)
            if f == 0:
                stage_out(cur)
            if f == 1:
                @pl.when(s >= 2)
                def _():
                    out_copy(s - 2, cur).start()
            if f == FO:
                stage_proj(sB, cur)
            if f == FN:
                stage_ln2(cur)
        return carry

    lax.fori_loop(1, NB + 1, body, 0)
    out_copy(NB - 3, (NB - 3) % 2).wait()
    stage_out((NB - 1) % 2)
    out_copy(NB - 1, (NB - 1) % 2).start()
    out_copy(NB - 2, (NB - 2) % 2).wait()
    out_copy(NB - 1, (NB - 1) % 2).wait()


@jax.jit
def pallas_adaLN_cond__sliding_local_dilated__dense_activation_relu__prompt_kernel(
    A_x: jax.Array,
    A_wqkv: jax.Array,
    A_wo: jax.Array,
    B_x: jax.Array,
    B_w1: jax.Array,
    B_w2: jax.Array,
    c: jax.Array,
    w_mod: jax.Array,
):
    del B_x
    anyspec = pl.BlockSpec(memory_space=pl.ANY)
    outT = pl.pallas_call(
        _kernel,
        grid=(1,),
        in_specs=[anyspec] * 7,
        out_specs=anyspec,
        out_shape=jax.ShapeDtypeStruct((D, S), bf16),
        scratch_shapes=[
            pltpu.VMEM((1, D), bf16),
            pltpu.VMEM((D, 6 * D), bf16),
            pltpu.VMEM((NB + 1, D, TM), bf16),
            pltpu.VMEM((2, D, TM), bf16),
            pltpu.VMEM((D, 3 * D), bf16),
            pltpu.VMEM((D, D), bf16),
            pltpu.VMEM((D, DFF), bf16),
            pltpu.VMEM((D, DFF), bf16),
            pltpu.VMEM((4 * D, 128), f32),
            pltpu.VMEM((5, 3 * D, 128), f32),
            pltpu.VMEM((NQ, KO), bf16),
            pltpu.VMEM((5, D, 128), f32),
            pltpu.VMEM((D, KO), bf16),
            pltpu.VMEM((NB, 5, TM, 128), bf16),
            pltpu.VMEM((2, 5, TM, 128), bf16),
            pltpu.VMEM((5, TM, 128), bf16),
            pltpu.VMEM((2, FC // 128, TM, 128), bf16),
            pltpu.VMEM((QKV_ROWS, 128), f32),
            pltpu.VMEM((2, NT, D, 128), f32),
            pltpu.VMEM((2, D, TM), f32),
            pltpu.VMEM((2, 8, D), f32),
            pltpu.SMEM((1,), jnp.int32),
            pltpu.SemaphoreType.DMA((9 + NB,)),
            pltpu.SemaphoreType.DMA((2,)),
        ],
        compiler_params=pltpu.CompilerParams(
            dimension_semantics=("arbitrary",),
            vmem_limit_bytes=110 * 1024 * 1024,
            flags={"XLA_TPU_EVENLY_DISTRIBUTE_CRITICAL_NODES": True},
        ),
    )(c, w_mod, A_x.reshape(S, D).T, A_wqkv, A_wo, B_w1, B_w2.T)
    return outT.T.reshape(1, S, D)
```

```python
import math

import jax
import jax.numpy as jnp
from jax import lax
import jax.experimental.pallas as pl
import jax.experimental.pallas.tpu as pltpu

S, D, H, DH, W, DIL, DFF = 2048, 576, 32, 18, 8, 2, 4608
TM = 256
FC = 512
RG = 16
NB = S // TM
NT = TM // 128
NF = DFF // FC
HALO = 16
NQ = 14 * 128
KO = 5 * 128
NC = W // 2
f32 = jnp.float32
bf16 = jnp.bfloat16
NTD = (((1,), (1,)), ((), ()))
QP = S + 16
KV0 = 5 * QP
KVP = HALO + S + 8
PIN0 = KV0 + NC * 9 * KVP
QKV_ROWS = PIN0 + 8
WCH = ((0, 640), (640, 1152), (1152, 3 * D))
FO, FN = 5, 7


def _qkv_row(s, d):
    if d < 16:
        return (0, 5, 9)[s] * 128 + d * 32
    return (4 * 128, 13 * 128, 13 * 128 + 64)[s] + (d - 16) * 32


def _mul(a, b):
    r = a * b
    if not isinstance(r, int):
        r = pl.multiple_of(r, b)
    return r


def _ld_tiles(ref, width):
    n = -(-width // 128)
    return jnp.concatenate([ref[t] for t in range(n)], axis=1)[:, 0:width]


def _st_tiles(ref, val):
    for t in range(-(-val.shape[1] // 128)):
        n = min(128, val.shape[1] - t * 128)
        ref[t, :, 0:n] = val[:, t * 128:t * 128 + n]


def _kernel(c_hbm, wmod_hbm, xT_hbm, wqkv_hbm, wo_hbm, w1_hbm, w2T_hbm, outT_hbm,
            c_v, wmod_v, x_v, out_v, wqkv_v, wo_v, w1_v, w2T_v,
            modT_v, wt32_v, wqkvT_v, wo32_v, woT_v,
            h_v, h2_v, o_v, hh_v, qkv_v, acc_v, x1_v, modS_v, z_ref, sem, osem):
    def cp(i, src, dst):
        return pltpu.make_async_copy(src, dst, sem.at[i])
    d_c = cp(0, c_hbm, c_v)
    d_modA = cp(1, wmod_hbm.at[:, pl.ds(0, 2 * D)], wmod_v.at[:, pl.ds(0, 2 * D)])
    d_modB = cp(2, wmod_hbm.at[:, pl.ds(2 * D, 4 * D)], wmod_v.at[:, pl.ds(2 * D, 4 * D)])
    d_wo = cp(3, wo_hbm, wo_v)
    d_w1 = cp(4, w1_hbm, w1_v)
    d_w2 = cp(5, w2T_hbm, w2T_v)
    d_wqkv = [cp(6 + i, wqkv_hbm.at[:, pl.ds(a, b - a)], wqkv_v.at[:, pl.ds(a, b - a)])
              for i, (a, b) in enumerate(WCH)]
    d_x = [cp(9 + b, xT_hbm.at[:, pl.ds(b * TM, TM)], x_v.at[b]) for b in range(NB)]
    for d in ([d_wqkv[0], d_c, d_modA, d_x[0], d_x[1], d_wqkv[1], d_wqkv[2]] + d_x[2:]
              + [d_wo, d_modB, d_w1, d_w2]):
        d.start()

    def out_copy(b, slot):
        return pltpu.make_async_copy(out_v.at[slot], outT_hbm.at[:, pl.ds(_mul(b, TM), TM)], osem.at[slot])

    def mod_rows(col0, ncol):
        c = c_v[...].astype(f32)
        s = (c * jax.nn.sigmoid(c)).astype(bf16)
        return jnp.dot(jnp.broadcast_to(s, (8, D)), wmod_v[:, col0:col0 + ncol], preferred_element_type=f32)

    def mod_first():
        m = mod_rows(0, 2 * D)
        modS_v[0] = m[:, 0:D]
        modS_v[1] = m[:, D:2 * D] + 1.0

    def mod_rest():
        m = mod_rows(2 * D, 4 * D)
        modS_v[2] = m[:, D:2 * D]
        modS_v[3] = m[:, 2 * D:3 * D] + 1.0
        modT_v[0] = jnp.broadcast_to(m[0:1, 0:D], (128, D)).T
        modT_v[1] = jnp.broadcast_to(m[0:1, 3 * D:4 * D], (128, D)).T

    def gate(j):
        return jnp.tile(modT_v[j], (1, NT))

    def build_wqkv(s):
        c0, c1 = WCH[s]
        wt = wqkv_v[:, c0:c1].T.astype(f32)
        for kt in range(5):
            n = min(128, D - kt * 128)
            blk = wt[:, kt * 128:kt * 128 + n]
            if n < 128:
                blk = jnp.concatenate([blk, jnp.zeros((c1 - c0, 128 - n), f32)], axis=1)
            wt32_v[kt, c0:c1, :] = blk
        if s == 0:
            wqkvT_v[4 * 128 + 64:5 * 128, :] = jnp.zeros((64, KO), bf16)
        for kt in range(5):
            for d in range(DH):
                rows = [wt32_v[kt, pl.ds(s * D + DH * 8 * hg + d, 8, stride=DH), :] for hg in range(4)]
                r0 = _qkv_row(s, d)
                wqkvT_v[r0:r0 + 32, kt * 128:(kt + 1) * 128] = jnp.concatenate(rows, axis=0).astype(bf16)

    def build_wo():
        w = wo_v[...].astype(f32)
        for nt in range(5):
            n = min(128, D - nt * 128)
            blk = w[:, nt * 128:nt * 128 + n]
            if n < 128:
                blk = jnp.concatenate([blk, jnp.zeros((D, 128 - n), f32)], axis=1)
            wo32_v[nt] = blk
        for nt in range(5):
            n = min(128, D - nt * 128)
            parts = []
            for t in range(5):
                for dd in range(4):
                    if t == 4 and dd < 2:
                        parts.append(jnp.zeros((32, 128), f32))
                        continue
                    d = 4 * t + dd if t < 4 else 14 + dd
                    parts += [wo32_v[nt, pl.ds(DH * 8 * hg + d, 8, stride=DH), :] for hg in range(4)]
            blk = jnp.concatenate(parts, axis=0).astype(bf16)
            woT_v[nt * 128:nt * 128 + n, :] = blk.T[0:n, :]

    def layer_norm(x, j, dst):
        g = jnp.tile(modS_v[j + 1], (2, 1))
        sh = jnp.tile(modS_v[j], (2, 1))
        for r in range(0, TM, 16):
            xf = x[r:r + 16, :].astype(f32)
            xc = xf - jnp.mean(xf, axis=1, keepdims=True)
            v = jnp.mean(xc * xc, axis=1, keepdims=True)
            _st_tiles(dst.at[:, r:r + 16, :], ((xc * lax.rsqrt(v + 1e-5)) * g + sh).astype(bf16))

    def stage_ln1(b, z=0):
        layer_norm(x_v[b + z].T, 0, h_v.at[b])

    cexp = (DH ** -0.5) * math.log2(math.e)

    def stage_qkv(b, t0=0, t1=14):
        r = b * TM
        qkv = lax.dot_general(_ld_tiles(h_v.at[b], D), wqkvT_v[t0 * 128:t1 * 128, 0:D], NTD,
                              preferred_element_type=f32)
        for t in range(t0, t1):
            val = qkv[:, (t - t0) * 128:(t - t0 + 1) * 128]
            if t == 0:
                x_v[NB, 0:16, 0:128] = val[0:16, :].astype(bf16)
            if t < 5:
                qkv_v[pl.ds(t * QP + r, TM), :] = val * cexp
            else:
                for cc in range(NC):
                    qkv_v[pl.ds(KV0 + (cc * 9 + t - 5) * KVP + HALO + DIL * cc + r, TM), :] = val

    def stage_attn(b, g):
        r0 = _mul(b, TM) + g * RG

        def windows(t):
            out = [None] * W
            for cc in range(NC):
                v = qkv_v[pl.ds(KV0 + (cc * 9 + t) * KVP + HALO - DIL * NC + r0, RG + DIL * NC), :]
                out[cc + NC] = v[0:RG]
                out[cc] = v[DIL * NC:DIL * NC + RG]
            return out

        ls = [None] * W
        for t in range(5):
            q = qkv_v[pl.ds(t * QP + r0, RG), :]
            kw = windows(t if t < 4 else 8)
            for w in range(W):
                p = q * kw[w]
                ls[w] = p if ls[w] is None else ls[w] + p
        for w in range(W):
            acc = ls[w] + pltpu.roll(ls[w], 64, 1)
            acc = acc + pltpu.roll(acc, 32, 1)
            if g * RG < DIL * w:
                row = r0 + lax.broadcasted_iota(jnp.int32, (RG, 128), 0)
                acc = jnp.where(row >= DIL * w, acc, -1e9)
            ls[w] = acc
        mx = ls[0]
        for w in range(1, W):
            mx = jnp.maximum(mx, ls[w])
        es = [jnp.exp2(l - mx) for l in ls]
        sm = es[0]
        for w in range(1, W):
            sm = sm + es[w]
        inv = 1.0 / sm
        for t in range(5):
            vw = windows(4 + t if t < 4 else 8)
            acc = es[0] * vw[0]
            for w in range(1, W):
                acc = acc + es[w] * vw[w]
            o_v[t, g * RG:(g + 1) * RG, :] = (acc * inv).astype(bf16)

    def stage_proj(b, slot):
        a = lax.dot_general(woT_v[...], _ld_tiles(o_v, KO), NTD, preferred_element_type=f32)
        x1_v[slot] = x_v[b].astype(f32) + gate(0) * a

    def stage_ln2(slot):
        layer_norm(x1_v[slot].T, 2, h2_v.at[slot])

    def stage_up(slot, f):
        hh = jnp.dot(_ld_tiles(h2_v.at[slot], D), w1_v[:, f * FC:(f + 1) * FC], preferred_element_type=f32)
        hh = jnp.maximum(hh, 0.0).astype(bf16)
        for t in range(FC // 128):
            hh_v[f % 2, t] = hh[:, t * 128:(t + 1) * 128]

    def stage_down(slot, f, behind):
        p = lax.dot_general(w2T_v[:, f * FC:(f + 1) * FC], _ld_tiles(hh_v.at[f % 2], FC), NTD,
                            preferred_element_type=f32)
        for j in range(NT):
            val = p[:, j * 128:(j + 1) * 128]
            if f == 0:
                acc_v[slot, j] = val
            else:
                acc_v[slot, j] += val
            if j == 0:
                qkv_v[PIN0:PIN0 + 8, :] = val[D - 8:D, :]
                behind()

    def stage_out(slot):
        acc = jnp.concatenate([acc_v[slot, j] for j in range(NT)], axis=1)
        out_v[slot] = (x1_v[slot] + gate(1) * acc).astype(bf16)

    nG = TM // RG
    z_ref[0] = 0
    for t in range(NC * 9):
        qkv_v[KV0 + t * KVP:KV0 + t * KVP + HALO + 8, :] = jnp.zeros((HALO + 8, 128), f32)
    for j in range(NT):
        acc_v[1, j] = jnp.zeros((D, 128), f32)
    x1_v[1] = jnp.zeros((D, TM), f32)
    d_wqkv[0].wait()
    build_wqkv(0)
    d_c.wait()
    d_modA.wait()
    mod_first()
    d_x[0].wait()
    stage_ln1(0)
    d_x[1].wait()
    stage_qkv(0, 0, 5)
    stage_ln1(1)
    d_wqkv[1].wait()
    d_wqkv[2].wait()
    stage_qkv(1, 0, 5)
    build_wqkv(1)
    stage_qkv(0, 5, 9)
    build_wqkv(2)
    stage_qkv(0, 9, 14)
    for b in range(2, NB):
        d_x[b].wait()
    d_wo.wait()
    z = z_ref[0]
    gi = 0
    stage_ln1(2)
    for b in range(1, NB - 1):
        stage_qkv(b, 5 if b == 1 else 0)
        if b + 2 < NB:
            stage_ln1(b + 2, z)
        if b == 1:
            build_wo()
        gend = min(nG, (nG * b) // (NB - 3))
        while gi < gend:
            stage_attn(z, gi)
            gi += 1
    d_modB.wait()
    d_w1.wait()
    d_w2.wait()
    mod_rest()
    stage_proj(0, 0)
    stage_qkv(NB - 1)
    stage_ln2(0)

    def body(s, carry):
        cur = s % 2
        prv = 1 - cur
        sB = jnp.minimum(s, NB - 1)

        @pl.when(s >= 4)
        def _():
            out_copy(s - 4, cur).wait()

        state = [0, 0]

        def attn():
            state[1] += 1
            gend = min(nG, (nG * state[1]) // FO)
            while state[0] < gend:
                stage_attn(sB, state[0])
                state[0] += 1

        stage_up(prv, 0)
        for f in range(NF):
            if f + 1 < NF:
                stage_up(prv, f + 1)
            stage_down(prv, f, attn)
            if f == 0:
                stage_out(cur)
            if f == 1:
                @pl.when(s >= 2)
                def _():
                    out_copy(s - 2, cur).start()
            if f == FO:
                stage_proj(sB, cur)
            if f == FN:
                stage_ln2(cur)
        return carry

    lax.fori_loop(1, NB + 1, body, 0)
    out_copy(NB - 3, (NB - 3) % 2).wait()
    stage_out((NB - 1) % 2)
    out_copy(NB - 1, (NB - 1) % 2).start()
    out_copy(NB - 2, (NB - 2) % 2).wait()
    out_copy(NB - 1, (NB - 1) % 2).wait()


@jax.jit
def pallas_adaLN_cond__sliding_local_dilated__dense_activation_relu__prompt_kernel(
    A_x: jax.Array,
    A_wqkv: jax.Array,
    A_wo: jax.Array,
    B_x: jax.Array,
    B_w1: jax.Array,
    B_w2: jax.Array,
    c: jax.Array,
    w_mod: jax.Array,
):
    del B_x
    anyspec = pl.BlockSpec(memory_space=pl.ANY)
    outT = pl.pallas_call(
        _kernel,
        grid=(1,),
        in_specs=[anyspec] * 7,
        out_specs=anyspec,
        out_shape=jax.ShapeDtypeStruct((D, S), bf16),
        scratch_shapes=[
            pltpu.VMEM((1, D), bf16),
            pltpu.VMEM((D, 6 * D), bf16),
            pltpu.VMEM((NB + 1, D, TM), bf16),
            pltpu.VMEM((2, D, TM), bf16),
            pltpu.VMEM((D, 3 * D), bf16),
            pltpu.VMEM((D, D), bf16),
            pltpu.VMEM((D, DFF), bf16),
            pltpu.VMEM((D, DFF), bf16),
            pltpu.VMEM((2, D, 128), f32),
            pltpu.VMEM((5, 3 * D, 128), f32),
            pltpu.VMEM((NQ, KO), bf16),
            pltpu.VMEM((5, D, 128), f32),
            pltpu.VMEM((D, KO), bf16),
            pltpu.VMEM((NB, 5, TM, 128), bf16),
            pltpu.VMEM((2, 5, TM, 128), bf16),
            pltpu.VMEM((5, TM, 128), bf16),
            pltpu.VMEM((2, FC // 128, TM, 128), bf16),
            pltpu.VMEM((QKV_ROWS, 128), f32),
            pltpu.VMEM((2, NT, D, 128), f32),
            pltpu.VMEM((2, D, TM), f32),
            pltpu.VMEM((4, 8, D), f32),
            pltpu.SMEM((1,), jnp.int32),
            pltpu.SemaphoreType.DMA((9 + NB,)),
            pltpu.SemaphoreType.DMA((2,)),
        ],
        compiler_params=pltpu.CompilerParams(
            dimension_semantics=("arbitrary",),
            vmem_limit_bytes=110 * 1024 * 1024,
            flags={"XLA_TPU_EVENLY_DISTRIBUTE_CRITICAL_NODES": True},
        ),
    )(c, w_mod, A_x.reshape(S, D).T, A_wqkv, A_wo, B_w1, B_w2.T)
    return outT.T.reshape(1, S, D)
```
